```python
import os as _os
_os.environ.setdefault('JAX_PLATFORMS', 'cpu')
import jax
import jax.numpy as jnp

def _softmax(x, axis=-1):
    return jax.nn.softmax(x, axis=axis)

def _gelu(x):
    return jax.nn.gelu(x, approximate=True)

def _silu(x):
    return jax.nn.silu(x)

def _sigmoid(x):
    return jax.nn.sigmoid(x)

def _layernorm(x, axis=-1, eps=1e-05):
    m = jnp.mean(x, axis=axis, keepdims=True)
    v = jnp.var(x, axis=axis, keepdims=True)
    return (x - m) / jnp.sqrt(v + eps)

def _scatter_add(tgt, idx, src, axis=0):
    return tgt.at[idx].add(src)

def _segment_sum(src, seg, n):
    return jax.ops.segment_sum(src, seg, n)

class _Rng:

    def __init__(self, key):
        self._k = key

    def _next(self):
        self._k, sub = jax.random.split(self._k)
        return sub

    def normal(self, shape):
        return jax.random.normal(self._next(), shape, dtype=jnp.bfloat16)

    def randint(self, lo, hi, shape):
        return jax.random.randint(self._next(), shape, lo, hi, dtype=jnp.int32)

    def uniform(self, shape, lo=0.0, hi=1.0):
        return jax.random.uniform(self._next(), shape, jnp.bfloat16, lo, hi)

    def permutation(self, n):
        return jax.random.permutation(self._next(), n)
kernel_name = 'adaLN_cond__mha_block__geglu_ffn__prompt'

def setup_inputs():
    _rng = _Rng(jax.random.key(int.from_bytes(__import__("os").urandom(4), "little")))
    _w = lambda a: (lambda t: t.astype(jnp.bfloat16) if jnp.issubdtype(t.dtype, jnp.floating) else t)(jnp.asarray(a))

    def _A_setup():
        B, S, D, H = (1, 2048, 640, 32)
        return {'x': _w((lambda *s: _rng.normal(s) * 0.05)(B, S, D)), 'wqkv': _w((lambda *s: _rng.normal(s) * 0.05)(D, 3 * D)), 'wo': _w((lambda *s: _rng.normal(s) * 0.05)(D, D))}
    _A_in = _A_setup()

    def _B_setup():
        B, S, D, F = (1, 2048, 640, 1728)
        return {'x': _w((lambda *s: _rng.normal(s) * 0.05)(B, S, D)), 'w_gate': _w((lambda *s: _rng.normal(s) * 0.05)(D, F)), 'w_up': _w((lambda *s: _rng.normal(s) * 0.05)(D, F)), 'w_down': _w((lambda *s: _rng.normal(s) * 0.05)(F, D))}
    _B_in = _B_setup()
    return {'A_x': _A_in['x'], 'A_wqkv': _A_in['wqkv'], 'A_wo': _A_in['wo'], 'B_x': _B_in['x'], 'B_w_gate': _B_in['w_gate'], 'B_w_up': _B_in['w_up'], 'B_w_down': _B_in['w_down'], 'c': _w((lambda *s: _rng.normal(s) * 0.05)(1, 640) * 8.0), 'w_mod': _w((lambda *s: _rng.normal(s) * 0.05)(640, 6 * 640) * 640 ** (-0.5) * 8.0)}

def reference(A_x, A_wqkv, A_wo, B_x, B_w_gate, B_w_up, B_w_down, c, w_mod):

    def _A_ref(x, wqkv, wo):
        B, S, D = x.shape
        H = 32
        Dh = D // H
        qkv = (lambda x, *d: x.transpose(*d))((x @ wqkv).reshape(B, S, 3, H, Dh), 2, 0, 3, 1, 4)
        q, k, v = (qkv[0], qkv[1], qkv[2])
        scores = jnp.einsum('bhqd,bhkd->bhqk', q, k) * Dh ** (-0.5)
        p = _softmax(scores, axis=-1)
        o = jnp.einsum('bhqk,bhkd->bhqd', p, v)
        return (lambda x, *d: x.transpose(*d))(o, 0, 2, 1, 3).reshape(B, S, D) @ wo

    def _B_ref(x, w_gate, w_up, w_down):
        return _gelu(x @ w_gate) * (x @ w_up) @ w_down
    x = A_x
    mod = (_silu(c) @ w_mod).reshape(c.shape[0], 6, 1, -1)
    sa, ca, ga, sb, cb, gb = (mod[:, 0].copy(), mod[:, 1].copy(), mod[:, 2].copy(), mod[:, 3].copy(), mod[:, 4].copy(), mod[:, 5].copy())
    h = _layernorm(x, axis=-1) * (1 + ca) + sa
    x = x + ga * _A_ref(h, A_wqkv, A_wo)
    h = _layernorm(x, axis=-1) * (1 + cb) + sb
    x = x + gb * _B_ref(h, B_w_gate, B_w_up, B_w_down)
    return x
```

```python
import math

import jax
import jax.numpy as jnp
import jax.experimental.pallas as pl
import jax.experimental.pallas.tpu as pltpu
from jax import lax

F32 = jnp.float32
BF16 = jnp.bfloat16

H = 32
EPS = 1e-5
QB = 512
KC = 128
LAG = 2
RB = 512

NN = (((1,), (0,)), ((), ()))
NT = (((1,), (1,)), ((), ()))
TN = (((0,), (0,)), ((), ()))


def _dot(a, b, dims=NN):
    return lax.dot_general(a, b, dims, preferred_element_type=F32)


def _ln_mod(x, scale1p, shift):
    inv_d = 1.0 / x.shape[-1]
    mean = jnp.sum(x, axis=-1, keepdims=True) * inv_d
    xc = x - mean
    var = jnp.sum(xc * xc, axis=-1, keepdims=True) * inv_d
    return (xc * lax.rsqrt(var + EPS) * scale1p + shift).astype(BF16)


def _geglu(g, u):
    c0 = math.sqrt(2.0 / math.pi)
    t = jnp.tanh(g * (c0 + (c0 * 0.044715) * (g * g)))
    hg = 0.5 * g
    return ((hg + hg * t) * u).astype(BF16)


def _kernel(c_ref, x_hbm, wqkv_hbm, wo_hbm, wgt_hbm, wut_hbm, wd_hbm, wmod_hbm,
            out_hbm,
            x_v, wqkv_v, wo_v, wgu_v, wd_v, wmod_v, out_v,
            wqt_s, wvt_s, h_s, k_s, q_s, v_s, s0, s1, ot_s, sems):
    S, D = x_v.shape
    FF = wd_v.shape[0]
    DH = D // H
    NP = H // 2
    PW = 2 * DH
    n_rb = S // RB
    n_qb = S // QB
    n_kc = S // KC
    f_main = FF // 128 * 128
    f_tail = FF - f_main

    def copy(src, dst, i):
        return pltpu.make_async_copy(src, dst, sems.at[i])

    cp_mod_a = copy(wmod_hbm.at[:, 0:2 * D], wmod_v.at[:, 0:2 * D], 0)
    cp_mod_b = copy(wmod_hbm.at[:, 2 * D:], wmod_v.at[:, 2 * D:], 1)
    cp_x = [copy(x_hbm.at[r * RB:(r + 1) * RB], x_v.at[r * RB:(r + 1) * RB], 2 + r)
            for r in range(n_rb)]
    b = 2 + n_rb
    cp_wqkv = copy(wqkv_hbm, wqkv_v, b)
    cp_wo = copy(wo_hbm, wo_v, b + 1)
    cp_wd = copy(wd_hbm, wd_v, b + 2)
    cp_wgu = [
        copy(wgt_hbm, wgu_v.at[0:FF], b + 3),
        copy(wut_hbm.at[f_main:FF], wgu_v.at[FF:FF + f_tail], b + 4),
        copy(wut_hbm.at[0:f_main], wgu_v.at[FF + f_tail:], b + 5),
    ]
    cp_out = [copy(out_v.at[r * RB:(r + 1) * RB], out_hbm.at[r * RB:(r + 1) * RB],
                   b + 6 + r) for r in range(n_rb)]

    cp_mod_a.start()
    cp_x[0].start()
    cp_wqkv.start()

    cc = c_ref[...].astype(F32)
    sc = cc / (1.0 + jnp.exp(-cc))
    sc = jnp.broadcast_to(sc, (16, D)).astype(BF16)
    cp_mod_a.wait()
    for r in range(1, n_rb):
        cp_x[r].start()
    mod_a = _dot(sc, wmod_v[:, 0:2 * D])[0:1]
    shift_a = mod_a[:, 0:D]
    scale_a = 1.0 + mod_a[:, D:2 * D]

    cp_x[0].wait()
    h_s[0] = _ln_mod(x_v[0:RB].astype(F32), scale_a, shift_a)
    cp_wqkv.wait()
    cp_mod_b.start()
    cp_wo.start()
    cp_wd.start()
    for cp in cp_wgu:
        cp.start()
    wqt_s[...] = wqkv_v[:, 0:D].T
    wvt_s[...] = wqkv_v[:, 2 * D:3 * D].T
    for r in range(1, n_rb):
        cp_x[r].wait()

    q_scale = DH ** -0.5 * math.log2(math.e)
    row8 = lax.broadcasted_iota(jnp.int32, (8, RB), 0)
    lo8 = row8 < (DH % 8)

    def qkv_block(r, carry):
        rows = pl.ds(pl.multiple_of(r * RB, RB), RB)
        h = h_s[r % 2]
        k = _dot(h, wqkv_v[:, D:2 * D]).astype(BF16)
        qt = _dot(wqt_s[...], h, NT) * q_scale
        vt = _dot(wvt_s[...], h, NT)
        zero8 = jnp.zeros((8, RB), F32)
        for p in range(NP):
            o = p * PW
            k_s[2 * p, rows, :] = k[:, o:o + 32]
            k_s[2 * p + 1, rows, :] = k[:, o + 8:o + 40]
            q_mid = qt[o + 16:o + 24]
            q_s[2 * p, r] = jnp.concatenate(
                [qt[o:o + 16], jnp.where(lo8, q_mid, 0.0), zero8], axis=0).astype(BF16)
            q_s[2 * p + 1, r] = jnp.concatenate(
                [zero8, jnp.where(lo8, 0.0, q_mid), qt[o + 24:o + 40]], axis=0).astype(BF16)
            v_mid = vt[o + 16:o + 24]
            v_s[2 * p, r] = jnp.concatenate(
                [vt[o:o + 16], jnp.where(lo8, v_mid, 1.0)], axis=0)
            v_s[2 * p + 1, r] = jnp.concatenate(
                [jnp.where(lo8, 1.0, v_mid), vt[o + 24:o + 40]], axis=0)
        r1 = jnp.minimum(r + 1, n_rb - 1)
        x1 = x_v[pl.ds(pl.multiple_of(r1 * RB, RB), RB), :].astype(F32)
        h_s[(r + 1) % 2] = _ln_mod(x1, scale_a, shift_a)
        return carry

    lax.fori_loop(0, n_rb, qkv_block, 0)

    sbuf = (s0, s1)

    def qk_slot(head, qb, c, buf, m):
        s = _dot(k_s[head, c * KC:(c + 1) * KC, :], q_s[head, qb])
        buf[c * KC:(c + 1) * KC, :] = s
        mm = jnp.max(s.reshape(KC // 8, 8, QB), axis=0)
        return mm if m is None else jnp.maximum(m, mm)

    def pv_slot(head, c, buf, m, acc):
        p = jnp.exp2(buf[c * KC:(c + 1) * KC, :] - m).astype(BF16)
        lo = c * KC % RB
        o = _dot(v_s[head, c * KC // RB, :, lo:lo + KC], p)
        return o if acc is None else acc + o

    def col_max(m):
        return jnp.max(m, axis=0, keepdims=True)

    m = None
    for c in range(n_kc):
        m = qk_slot(0, 0, c, s0, m)
    m_cur = col_max(m)
    m = None
    for c in range(LAG):
        m = qk_slot(1, 0, c, s1, m)

    QPI = 2
    n_it = NP * n_qb // QPI

    def attn_body(j, carry):
        m_cur, m = carry
        for t in range(QPI):
            i = j * QPI + t
            pair, qb = i // n_qb, i % n_qb
            i2 = jnp.minimum(i + 1, NP * n_qb - 1)
            pair2, qb2 = i2 // n_qb, i2 % n_qb
            accs = []
            for u in range(2):
                nxt = (2 * pair + 1, qb) if u == 0 else (2 * pair2, qb2)
                nxt2 = (2 * pair2, qb2) if u == 0 else (2 * pair2 + 1, qb2)
                acc = None
                for c in range(n_kc):
                    if c + LAG < n_kc:
                        m = qk_slot(*nxt, c + LAG, sbuf[1 - u], m)
                        if c + LAG == n_kc - 1:
                            m_nxt, m = col_max(m), None
                    else:
                        m = qk_slot(*nxt2, c + LAG - n_kc, sbuf[u], m)
                    acc = pv_slot(2 * pair + u, c, sbuf[u], m_cur, acc)
                m_cur = m_nxt
                accs.append(acc)
            ae, ao = accs
            ae = ae * (1.0 / ae[DH:DH + 1])
            ao = ao * (1.0 / ao[0:1])
            ot_s[qb, pair] = jnp.concatenate(
                [ae[0:16], jnp.where(lo8, ae[16:24], ao[0:8]), ao[8:24]], axis=0)
        return m_cur, m

    lax.fori_loop(0, n_it, attn_body, (m_cur, m))

    cp_mod_b.wait()
    mod_b = _dot(sc, wmod_v[:, 2 * D:])[0:1]
    gate_a = mod_b[:, 0:D]
    shift_b = mod_b[:, D:2 * D]
    scale_b = 1.0 + mod_b[:, 2 * D:3 * D]
    gate_b = mod_b[:, 3 * D:4 * D]
    cp_wo.wait()
    cp_wd.wait()
    for cp in cp_wgu:
        cp.wait()

    def ffn_block(r, carry):
        rows = pl.ds(pl.multiple_of(r * RB, RB), RB)
        ot = ot_s[r].reshape(D, RB).astype(BF16)
        x1 = x_v[rows, :].astype(F32) + gate_a * _dot(ot, wo_v[...], TN)
        h2 = _ln_mod(x1, scale_b, shift_b)
        g = _dot(h2, wgu_v[0:f_main], NT)
        gu = _dot(h2, wgu_v[f_main:FF + f_tail], NT)
        u = _dot(h2, wgu_v[FF + f_tail:], NT)
        a = _geglu(g, u)
        a_tail = _geglu(gu[:, 0:f_tail], gu[:, f_tail:])
        y = _dot(a, wd_v[0:f_main]) + _dot(a_tail, wd_v[f_main:FF])
        out_v[rows, :] = (x1 + gate_b * y).astype(BF16)
        pltpu.make_async_copy(out_v.at[rows], out_hbm.at[rows],
                              sems.at[b + 6 + r]).start()
        return carry

    lax.fori_loop(0, n_rb, ffn_block, 0)
    for cp in cp_out:
        cp.wait()


@jax.jit
def pallas_adaLN_cond__mha_block__geglu_ffn__prompt_kernel(
    A_x: jax.Array,
    A_wqkv: jax.Array,
    A_wo: jax.Array,
    B_x: jax.Array,
    B_w_gate: jax.Array,
    B_w_up: jax.Array,
    B_w_down: jax.Array,
    c: jax.Array,
    w_mod: jax.Array,
):
    del B_x
    B, S, D = A_x.shape
    assert B == 1
    FF = B_w_down.shape[0]
    DH = D // H
    assert DH == 20 and RB == QB and S % RB == 0
    hbm = pl.BlockSpec(memory_space=pl.ANY)
    vmem = pltpu.VMEM
    out = pl.pallas_call(
        _kernel,
        out_shape=jax.ShapeDtypeStruct((S, D), A_x.dtype),
        in_specs=[pl.BlockSpec(memory_space=vmem)] + [hbm] * 7,
        out_specs=hbm,
        scratch_shapes=[
            vmem((S, D), BF16),
            vmem((D, 3 * D), BF16),
            vmem((D, D), BF16),
            vmem((2 * FF, D), BF16),
            vmem((FF, D), BF16),
            vmem((D, 6 * D), BF16),
            vmem((S, D), BF16),
            vmem((D, D), BF16),
            vmem((D, D), BF16),
            vmem((2, RB, D), BF16),
            vmem((H, S, 32), BF16),
            vmem((H, S // QB, 32, QB), BF16),
            vmem((H, S // RB, 24, RB), F32),
            vmem((S, QB), F32),
            vmem((S, QB), F32),
            vmem((S // QB, H // 2, 2 * DH, QB), F32),
            pltpu.SemaphoreType.DMA((8 + 2 * (S // RB),)),
        ],
        compiler_params=pltpu.CompilerParams(vmem_limit_bytes=110 * 1024 * 1024),
        name="adaln_mha_geglu_block",
    )(c, A_x.reshape(S, D), A_wqkv, A_wo, B_w_gate.T, B_w_up.T, B_w_down, w_mod)
    return out.reshape(B, S, D)
```

```python
import functools
import math

import numpy as np
import jax
import jax.numpy as jnp
import jax.experimental.pallas as pl
import jax.experimental.pallas.tpu as pltpu
from jax import lax

F32 = jnp.float32
BF16 = jnp.bfloat16

H = 32
EPS = 1e-5
RB = 512
HB = RB // 2
KC = 128
DS = 256
NV = 320
NV0 = 288
KS = 256

SUM_MIN = 2.0 ** -40
SUM_MAX = 2.0 ** 100
FINITE = float(np.finfo(np.float32).max)

NN = (((1,), (0,)), ((), ()))
NT = (((1,), (1,)), ((), ()))


def _dot(a, b, dims=NN):
    return lax.dot_general(a, b, dims, preferred_element_type=F32)


def _pack(v):
    return pltpu.bitcast(v.astype(BF16), F32)


def _unpack(v):
    return pltpu.bitcast(v, BF16)


def _rows(start, n):
    return pl.ds(pl.multiple_of(start, n), n)


def _layernorm(x):
    inv_d = 1.0 / x.shape[-1]
    xc = x - jnp.sum(x, axis=-1, keepdims=True) * inv_d
    var = jnp.sum(xc * xc, axis=-1, keepdims=True) * inv_d
    return xc * lax.rsqrt(var + EPS)


def _geglu(g, u):
    c0 = math.sqrt(2.0 / math.pi)
    t = jnp.tanh(g * (c0 + (c0 * 0.044715) * (g * g)))
    hg = 0.5 * g
    return (hg + hg * t) * u


def _strassen_lhs(a11, a12, a21, a22):
    return a11 + a22, a21 + a22, a11, a22, a11 + a12, a21 - a11, a12 - a22


def _strassen_rhs(b11, b12, b21, b22):
    return b11 + b22, b11, b12 - b22, b21 - b11, b22, b11 + b12, b21 + b22


def _token_operands(a11, a12, a21, a22, tail1, tail2):
    return _strassen_lhs(a11, a12, a21, a22) + (tail1, tail2, a12, a21)


STRASSEN_ORDER = (2, 4, 1, 3, 0, 6, 5)
STRASSEN_OUT = {
    4: (0, 1, lambda m: m[2] + m[4]),
    3: (1, 0, lambda m: m[1] + m[3]),
    6: (0, 0, lambda m: m[0] + m[3] - m[4] + m[6]),
    5: (1, 1, lambda m: m[0] - m[1] + m[2] + m[5]),
}


def _jobs(ref, fn, n, *args):
    return [(ref, functools.partial(fn, *args, e)) for e in range(0, n, 16)]


def _merge(*lists):
    keyed = [((i + 0.5) / len(l), j, v) for j, l in enumerate(lists) for i, v in enumerate(l)]
    return [v for _, _, v in sorted(keyed, key=lambda t: t[:2])]


def _kernel(c_hbm, x_hbm, wqkv_hbm, wo_hbm, wgt_hbm, wut_hbm, wd_hbm, wmod_hbm, out_hbm,
            p0, p1, y_s, x_v, wqkv_v, wgu_v, wd_v, wmod_v,
            k_s, qe_s, qo_s, qf_s, v_s, zero_s, o_s, ru_s, rd_s, sems):
    S, D = x_v.shape
    FF = wd_hbm.shape[0]
    DH = D // H
    NP = H // 2
    PW = 2 * DH
    n_rb = S // RB
    n_kc = S // KC
    n_qt = RB // 128
    n_ft = FF // 128
    f_tail = FF - n_ft * 128
    n_fp = (n_ft + 1) // 2

    def copy(src, dst, sem):
        return pltpu.make_async_copy(src, dst, sems.at[sem])

    def cols(src, dst, lo, hi, sem):
        return copy(src.at[:, lo:hi], dst.at[:, lo:hi], sem)

    cp_x = [copy(x_hbm.at[lo * HB:hi * HB], x_v.at[lo * HB:hi * HB], sem)
            for sem, (lo, hi) in enumerate(((0, 2), (2, 3), (3, 4), (4, 6), (6, 8)))]
    cp_scale = cols(wmod_hbm, wmod_v, D, 2 * D, 5)
    cp_wk = [cols(wqkv_hbm, wqkv_v, D, D + KS, 6), cols(wqkv_hbm, wqkv_v, D + KS, 2 * D, 7)]
    cp_qv = [cols(wmod_hbm, wmod_v, 0, D, 8), cols(wqkv_hbm, wqkv_v, 0, D, 8),
             cols(wqkv_hbm, wqkv_v, 2 * D, 3 * D, 8)]
    cp_ffn = [copy(wd_hbm, wd_v.at[0:FF], 9)]
    for t in range(n_ft + 1):
        n = 128 if t < n_ft else f_tail
        cp_ffn.append(copy(wgt_hbm.at[t * 128:t * 128 + n], wgu_v.at[t * 256:t * 256 + n], 9))
        cp_ffn.append(copy(wut_hbm.at[t * 128:t * 128 + n],
                           wgu_v.at[t * 256 + n:t * 256 + 2 * n], 9))
    sem_late, sem_out = 10, 11

    def start(c_v):
        cp_c = copy(c_hbm, c_v, 0)
        for cp in [cp_c, cp_x[0], cp_scale] + cp_wk + cp_x[1:] + cp_qv + cp_ffn:
            cp.start()
        cp_c.wait()
        cp_x[0].wait()
        return c_v[...].astype(F32)

    cc = pl.run_scoped(start, pltpu.VMEM((1, D), BF16))
    sc = jnp.broadcast_to(cc / (1.0 + jnp.exp(-cc)), (8, D))

    def hidden_zero(n):
        return ((n * (n + 1)) & 1) * n

    seed = jnp.max(cc[:, 0:128]).astype(jnp.int32)
    zero0 = hidden_zero(seed)
    marks = {}

    def paced(results, work):
        pieces = [(v, r) for v in results for r in range(0, v.shape[0], 8)]
        for i, (ref, fn) in enumerate(work):
            v, r = pieces[len(pieces) * i // len(work)]
            mark = lax.slice(v, (r, 0), (r + 8, 128))
            if ref is None:
                fn(mark)
                continue
            k = marks[id(ref)] = marks.get(id(ref), -1) + 1
            *idx, e = map(int, np.unravel_index(k, ref.shape[:-2] + (64,), order="F"))
            e = ref.shape[-2] - 8 - 8 * e
            ref[(*idx, slice(e, e + 8), slice(0, 128))] = mark
            fn()

    def tail_operand(ref):
        return jnp.concatenate(
            [ref[7 + half, 0:HB // 2, 3 * DS - D:] for half in range(2)], axis=0)

    def plain_operand(ref):
        head = jnp.concatenate([
            jnp.concatenate([ref[i, 0:HB // 2] for i in pair], axis=1)
            for pair in ((2, 9), (10, 3))], axis=0)
        return jnp.concatenate([head, tail_operand(ref)], axis=1)

    n_kb = NV // 8 * DH

    def kb_pos(i):
        return n_rb * S // 8 + i // n_qt, slice(i % n_qt * 128, (i % n_qt + 1) * 128)

    def kb_store(ref, zero, pair, odd, g, d):
        col = d + (DH if odd else 0)
        val = jnp.broadcast_to(k_s[pair, g * 4:g * 4 + 8, col:col + 1], (8, 128))
        for i, v in enumerate(lax.split(_unpack(val).astype(F32), [8, 8], 0)):
            row, cs = kb_pos((g + i) * DH + d)
            ref[lax.add(zero, np.int32(row)), :, cs] = v

    def project(xn_s, h0_s, wt_s, wqv_s, hq0_s, hq1_s, hq2_s):
        q_scale = DH ** -0.5 * math.log2(math.e)

        def norm0(r, e):
            xn = _layernorm(x_v[r * RB + 2 * e:r * RB + 2 * e + 32].astype(F32))
            xn_s[zero0 + r, 2 * e:2 * e + 32] = xn
            h0_s[r * HB + e:r * HB + e + 16] = _pack(xn * scale_a)

        def norm1(r, ref, slot, e):
            h1, h2 = (xn_s[r, half * HB + e:half * HB + e + 16] * scale_a + shift_a
                      for half in range(2))
            ops = _strassen_rhs(h1[:, 0:DS], h2[:, 0:DS], h1[:, DS:2 * DS], h2[:, DS:2 * DS])
            for i, v in enumerate(ops + (h1[:, D - DS:], h2[:, D - DS:])):
                ref[zero0 + slot, i, e // 2:e // 2 + 8] = _pack(v)

        def k_windows(r, e):
            k = _pack(y_s[_rows(r * RB + 2 * e, 32), :] + k_shift)
            lane = lax.broadcasted_iota(jnp.int32, (16, 128), 1)
            for p in range(NP):
                t, a = divmod(p * PW, 128)
                w = k[:, t * 128:(t + 1) * 128]
                if a + PW > 128:
                    w = jnp.where(lane < a, k[:, (t + 1) * 128:(t + 2) * 128], w)
                k_s[zero0 + p, _rows(r * HB + e, 16), :] = pltpu.roll(w, 128 - a, 1) if a else w

        def transpose_w(i, t):
            lo = 2 * i * D + t * 128
            wt = pltpu.bitcast(wqkv_v[:, lo:lo + 128].T, F32)
            for e in range(0, 128, 64):
                a, row = divmod(t * 128 + e, D // 2)
                row = (i * D // 2 + row) // 2
                wt_s[zero0 + a, row:row + 32] = wt[e // 2:e // 2 + 32]

        def prep_qv(r):
            top, bot = (_unpack(wt_s[a, r // 2:r // 2 + 8, 0:2 * DS]).astype(F32)
                        for a in range(2))
            for i, v in enumerate(_strassen_lhs(top[:, 0:DS], top[:, DS:],
                                                bot[:, 0:DS], bot[:, DS:])):
                wqv_s[zero0 + i, r // 2:r // 2 + 8] = _pack(v)

        def prep_kb(d, mark):
            row, cs = kb_pos(n_kb + d)
            p1[row, :, cs] = mark
            for g in range(0, NV0 // 8, 2):
                kb_store(p1, zero0, 0, False, g, d)

        def prep_up(p, r):
            one, two = (wgu_v[_rows(p * 512 + i * 256 + r, 16), 0:2 * DS].astype(F32)
                        for i in range(2))
            for i, v in enumerate(_strassen_rhs(one[:, 0:DS], two[:, 0:DS],
                                                one[:, DS:], two[:, DS:])):
                ru_s[zero0 + i, _rows(p * 128 + r // 2, 8), :] = _pack(v)

        def prep_down(half, p, r):
            r = half * 64 + r
            one, two = (wd_v[_rows(p * 256 + i * 128 + r, 16), 0:2 * DS].astype(F32)
                        for i in range(2))
            for i, v in enumerate(_strassen_rhs(one[:, 0:DS], one[:, DS:],
                                                two[:, 0:DS], two[:, DS:])):
                rd_s[zero0 + i, _rows(p * 64 + r // 2, 8), :] = _pack(v)

        def k_part(row, n, lo, hi, work=()):
            kf = [_dot(_unpack(h0_s[i // 2:i // 2 + 64]), wqkv_v[:, D + lo:D + hi])
                  for i in range(row, row + n, 128)]
            paced(kf, work)
            for i, v in enumerate(kf):
                y_s[row + i * 128:row + (i + 1) * 128, lo:hi] = v

        def qv_emit(r, a, b, qv):
            cs = slice(b * HB, (b + 1) * HB)
            qt, vt = qv[0:D // 2] * q_scale, qv[D // 2:]
            zeros = jnp.zeros((8, HB), F32)
            even = lax.broadcasted_iota(jnp.int32, (8, HB), 0) < DH % 8
            for i in range(NP // 2):
                p, o = a * NP // 2 + i, i * PW
                q_mid, v_mid = qt[o + 16:o + 24], vt[o + 16:o + 24]
                qe_s[p, r, :, cs] = _pack(jnp.concatenate(
                    [qt[o:o + 16], jnp.where(even, q_mid, 0.0), zeros], axis=0))
                qo_s[p, r, :, cs] = _pack(jnp.concatenate(
                    [zeros, zeros, jnp.where(even, 0.0, q_mid), qt[o + 24:o + 40], zeros], axis=0))
                qf_s[p, r, :, cs] = qt[o:o + PW]
                v_s[2 * p, r, :, cs] = jnp.concatenate(
                    [vt[o:o + 16], jnp.where(even, v_mid, 1.0)], axis=0)
                v_s[2 * p + 1, r, :, cs] = jnp.concatenate(
                    [jnp.where(even, 1.0, v_mid), vt[o + 24:o + 40]], axis=0)

        def qv_block(r, hq, work, early=()):
            work = _merge(work, _jobs(k_s, k_windows, HB, r))
            m, rest = {}, {}

            def last_columns(a):
                return _dot(_unpack(wt_s[a, 0:D // 2, 2 * DS:]), _unpack(tail_operand(hq)), NT)

            if early:
                rest = {a: last_columns(a) for a in range(2)}
                paced(list(rest.values()), early)
            for n, i in enumerate(STRASSEN_ORDER):
                m[i] = _dot(_unpack(wqv_s[i, 0:D // 2]), _unpack(hq[i, 0:HB // 2]), NT)
                paced([m[i]], work[len(work) * n // 7:len(work) * (n + 1) // 7])
                if i in STRASSEN_OUT:
                    a, b, combine = STRASSEN_OUT[i]
                    if a not in rest:
                        rest[a] = last_columns(a)
                    qv_emit(r, a, b, combine(m) + rest[a][:, b * HB:(b + 1) * HB])

        xn_s[0, 0:RB] = _layernorm(x_v[0:RB].astype(F32))
        cp_scale.wait()
        scale_a = 1.0 + _dot(sc, wmod_v[:, D:2 * D])[0:1]
        h0_s[0:HB] = _pack(xn_s[0, 0:RB] * scale_a)
        norm = [_jobs(xn_s, norm0, HB, r) for r in range(n_rb)]
        n = HB // 32
        cp_wk[0].wait()
        k_part(0, RB, 0, KS)
        cp_wk[1].wait()
        k_part(0, HB, KS, D)
        cp_x[1].wait()
        k_part(HB, HB, KS, D, norm[1][:n])
        cp_x[2].wait()
        k_part(RB, HB, 0, D, norm[1][n:])
        cp_x[3].wait()
        k_part(RB + HB, HB, 0, D, norm[2][:n])
        cp_x[4].wait()
        k_part(2 * RB, HB, 0, D, norm[2][n:] + norm[3][:n // 2])
        k_part(2 * RB + HB, HB, 0, D, norm[3][n // 2:])
        for cp in cp_qv:
            cp.wait()
        shift_a = _dot(sc, wmod_v[:, 0:D])
        k_part(3 * RB, HB, 0, D, [(wt_s, functools.partial(transpose_w, i, t))
                                  for i in range(2) for t in range(D // 128)])
        k_shift = _dot(shift_a, wqkv_v[:, D:2 * D])[0:1]
        shift_a = shift_a[0:1]
        prep = _jobs(wqv_s, prep_qv, D)
        k_part(3 * RB + HB, HB, 0, D,
               _merge(prep[:len(prep) // 3], _jobs(hq0_s, norm1, HB, 0, hq0_s, 0)))
        qv_block(0, hq0_s.at[0],
                 _jobs(hq1_s, norm1, HB, 1, hq1_s, 0) + _jobs(hq2_s, norm1, HB, 2, hq2_s, 0),
                 prep[len(prep) // 3:])
        qv_block(1, hq1_s.at[0], _jobs(hq2_s, norm1, HB, 3, hq2_s, 1)
                 + [(None, functools.partial(prep_kb, d)) for d in range(DH)])
        for cp in cp_ffn:
            cp.wait()
        wd_v[FF:] = jnp.zeros((wd_v.shape[0] - FF, D), BF16)

        def late_block(i, carry):
            n = (n_fp - 1) // 2
            qv_block(i + 2, hq2_s.at[i], _merge(
                [j for p in range(n) for j in _jobs(ru_s, prep_up, 256, i * n + p)],
                [j for p in range(n_fp) for j in _jobs(rd_s, prep_down, 64, i, p)]))
            return carry

        lax.fori_loop(0, 2, late_block, 0)

    pl.run_scoped(
        project,
        pltpu.VMEM((n_rb, RB + 96, D), F32),
        pltpu.VMEM((S // 2, D), F32),
        pltpu.VMEM((2, D // 2 + 64, D), F32),
        pltpu.VMEM((7, D // 2 + 48, DS), F32),
        pltpu.VMEM((1, 9, HB // 2 + 16, DS), F32),
        pltpu.VMEM((1, 9, HB // 2 + 16, DS), F32),
        pltpu.VMEM((2, 9, HB // 2 + 16, DS), F32),
    )

    zero_s[...] = jnp.zeros(zero_s.shape, F32)
    even_rows = lax.broadcasted_iota(jnp.int32, (8, RB), 0) < DH % 8

    def pv_tile(head, qb, c, pr, acc, dtype=F32):
        g = (qb * S + c * KC) // 8
        p = pr[g:g + KC // 8].reshape(KC, RB).astype(dtype)
        r, lo = divmod(c * KC, RB)
        return acc + _dot(v_s[head, r, :, lo:lo + KC], p)

    def phase(head, odd, pr, pw, first=False):
        zero = zero0 if first else hidden_zero(head)
        keep = lax.broadcasted_iota(jnp.int32, (8, 128), 0) >= zero
        pair1 = (head + 1) // 2
        pair2 = jnp.minimum((head + 2) // 2, NP - 1)
        q_s = qe_s if odd else qo_s
        nv = NV0 if first else NV
        bounds = [nv + (S - nv) // 16 * c // n_kc * 16 for c in range(n_kc + 1)]
        n_pieces = (S - nv) // 8 + (0 if first else 3 * n_kc)
        scores = [(g, t) for t in range(n_qt) for g in range(nv // 8)]
        columns = [(g, d) for d in range(DH) for g in range(0, NV // 8, 2)]
        state = {"offset": zero}

        def vector_scores(qb, g, t):
            if g == 0:
                rows = [jnp.broadcast_to(qf_s[pair1, qb, d:d + 1, t * 128:(t + 1) * 128], (8, 128))
                        for d in (range(DH) if odd else range(DH, PW))]
                state["q"] = [lax.concatenate(rows[i:i + n_qt], 1) for i in range(0, DH, n_qt)]
            state["offset"] = lax.add(state["offset"], zero)
            n = DH // n_qt
            k = pr[pl.ds(lax.add(state["offset"], np.int32(kb_pos(g * DH)[0])), n)]
            part = None
            for kv, qv in zip(lax.split(k.reshape(n * 8, RB), [8] * n, 0), state["q"]):
                prod = lax.mul(kv, qv)
                part = prod if part is None else lax.add(part, prod)
            return functools.reduce(lax.add, lax.split(part, [128] * n_qt, 1))

        for qb in range(n_rb):
            share = columns[len(columns) * qb // n_rb:len(columns) * (qb + 1) // n_rb]
            done = [0, 0, 0]

            def fill(piece):
                done[0] += 1
                while (done[1] + 0.9) * n_pieces <= done[0] * len(scores):
                    g, t = scores[done[1]]
                    done[1] += 1
                    s = lax.select(keep, vector_scores(qb, g, t),
                                   lax.slice(piece, (0, t * 128), (8, (t + 1) * 128)))
                    pw[lax.add(zero, np.int32(qb * S // 8 + g)), :, t * 128:(t + 1) * 128] = (
                        lax.exp2(s))
                while (done[2] + 0.5) * n_pieces <= done[0] * len(share):
                    kb_store(pw, zero, pair2, odd, *share[done[2]])
                    done[2] += 1

            acc = zero_s[...]
            for c in range(n_kc):
                k = k_s[pair1, bounds[c] // 2:bounds[c + 1] // 2, 0:2 * q_s.shape[2]]
                s = _dot(_unpack(k), _unpack(q_s[pair1, qb]))
                for i, piece in enumerate(lax.split(s, [8] * (s.shape[0] // 8), 0)):
                    pw[(qb * S + bounds[c]) // 8 + i] = lax.exp2(piece)
                    fill(piece)
                if not first:
                    acc = pv_tile(head, qb, c, pr, acc)
                    for piece in lax.split(acc, [8] * 3, 0):
                        fill(piece)
            assert done[1:] == [len(scores), len(share)]
            if not first:
                o_s[qb, head] = acc

    def normalised(even, odd):
        total = jnp.where(even_rows, odd[0:8], even[16:24])
        inv = pl.reciprocal(total, approx=True)
        inv = inv * (2.0 - total * inv)
        inv_even, inv_odd = inv[7:8], inv[0:1]
        mid = (jnp.where(even_rows, even[16:24], odd[0:8])
               * jnp.where(even_rows, inv_even, inv_odd))
        return jnp.concatenate([even[0:16] * inv_even, mid, odd[8:24] * inv_odd], axis=0), total

    def in_range(pairs):
        check = functools.reduce(jnp.add, [o[e:e + 8] for o, _ in pairs for e in range(0, PW, 8)])
        totals = [total for _, total in pairs]
        return ((jnp.abs(check) <= FINITE)
                & (functools.reduce(jnp.minimum, totals) >= SUM_MIN)
                & (functools.reduce(jnp.maximum, totals) <= SUM_MAX))

    def any_false(flags):
        return jnp.min(jnp.where(functools.reduce(jnp.logical_and, flags), 1.0, 0.0)) == 0.0

    def recompute_with_max(i, carry):
        pair, qb = i // n_rb, i % n_rb

        @pl.when(any_false([in_range([normalised(o_s[qb, 2 * pair], o_s[qb, 2 * pair + 1])])]))
        def _():
            for head, q_s in ((2 * pair, qe_s), (2 * pair + 1, qo_s)):
                def scores(r):
                    return _dot(_unpack(k_s[pair, _rows(r * HB, HB), 0:2 * q_s.shape[2]]),
                                _unpack(q_s[pair, qb]))

                top = lax.fori_loop(
                    0, n_rb,
                    lambda r, m: jnp.maximum(m, jnp.max(scores(r), axis=0, keepdims=True)),
                    jnp.full((1, RB), -jnp.inf, F32))
                o_s[qb, head] = lax.fori_loop(
                    0, n_rb,
                    lambda r, acc: acc + _dot(v_s[head, r],
                                              jnp.exp2(scores(r) - top).astype(BF16)),
                    jnp.zeros((24, RB), F32))
        return carry

    def finish(lu_s, ld_s, lo_s, ro_s, out_v, wmodb_v, wo_v):
        cp_late = [copy(wmod_hbm.at[:, 2 * D:], wmodb_v, sem_late), copy(wo_hbm, wo_v, sem_late)]

        def head_pair(pair, carry):
            phase(2 * pair, False, p0, p1)

            @pl.when(pair < NP - 1)
            def _():
                phase(2 * pair + 1, True, p1, p0)

            @pl.when(pair == 1)
            def _():
                for cp in cp_late:
                    cp.start()
            return carry

        phase(-1, True, p1, p0, first=True)
        lax.fori_loop(0, NP, head_pair, 0)
        for cp in cp_late:
            cp.wait()

        def last_head(qb, n):
            acc = zero_s[...]
            for c in range(n_kc):
                acc = pv_tile(H - 1, qb, c, p1, acc, BF16)
                if c == n_kc - 1:
                    o_s[qb, H - 1] = acc
                if (c + 1) * n // n_kc > c * n // n_kc:
                    yield acc

        def prep_wo(r):
            one, two = (wo_v[i * DS + r:i * DS + r + 16, 0:2 * DS].astype(F32) for i in range(2))
            for i, v in enumerate(_strassen_rhs(one[:, 0:DS], one[:, DS:],
                                                two[:, 0:DS], two[:, DS:])):
                ro_s[zero0 + i, r // 2:r // 2 + 8] = _pack(v)

        def norm2(r, slot, e):
            h1, h2 = (_layernorm(y_s[_rows(r * RB + half * HB + e, 16), :]) * scale_b + shift_b
                      for half in range(2))
            ops = [_pack(v) for v in _token_operands(
                h1[:, 0:DS], h1[:, DS:2 * DS], h2[:, 0:DS], h2[:, DS:2 * DS],
                h1[:, D - DS:], h2[:, D - DS:])]
            for i, v in enumerate(ops):
                lu_s[slot, i, _rows(e // 2, 8), :] = v
            return ops[0][:, 0:128]

        accs, mod = [], []
        for i, acc in enumerate(last_head(0, 4)):
            accs.append(acc)
            mod.append(_dot(sc, wmodb_v[:, i * D:(i + 1) * D])[0:1])
        paced(accs, _jobs(ro_s, prep_wo, DS))
        gate_a, shift_b, scale_b, gate_b = mod
        scale_b = 1.0 + scale_b

        safe = []
        for r in range(n_rb):
            steps = last_head(r + 1, 8) if r + 1 < n_rb else iter(range(8))
            pairs = [normalised(o_s[r, 2 * p], o_s[r, 2 * p + 1]) for p in range(NP)]
            safe.append(in_range(pairs))
            ot = jnp.concatenate([o for o, _ in pairs], axis=0)
            for i, v in enumerate(_token_operands(
                    ot[0:DS, 0:HB], ot[DS:2 * DS, 0:HB], ot[0:DS, HB:], ot[DS:2 * DS, HB:],
                    ot[2 * DS:, 0:HB], ot[2 * DS:, HB:])):
                lo_s[r % 2, i, :, DS - v.shape[0]:] = pltpu.bitcast(v.astype(BF16).T, F32)
            lo = lo_s.at[r % 2]

            def add_attention(r0, c0, y):
                rows = slice(r * RB + r0, r * RB + r0 + y.shape[0])
                cs = slice(c0, c0 + y.shape[1])
                y_s[rows, cs] = x_v[rows, cs].astype(F32) + gate_a[:, cs] * y

            next(steps)
            rest = _dot(_unpack(tail_operand(lo)), wo_v[2 * DS:, 0:2 * DS])
            add_attention(0, 2 * DS, _dot(_unpack(plain_operand(lo)), wo_v[:, 2 * DS:]))
            m = {}
            for n, i in enumerate(STRASSEN_ORDER):
                next(steps)
                m[i] = _dot(_unpack(lo[i]), _unpack(ro_s[i, 0:DS // 2]))
                k = HB // 16 + 1 - (n_rb - r) * len(STRASSEN_ORDER) + n
                if 0 <= k < HB // 16:
                    lo_s[zero0 + 2, k // 8, k % 8 * 8:k % 8 * 8 + 8, 0:128] = norm2(0, 0, k * 16)
                if i in STRASSEN_OUT:
                    a, b, combine = STRASSEN_OUT[i]
                    add_attention(a * HB, b * DS,
                                  combine(m) + rest[a * HB:(a + 1) * HB, b * DS:(b + 1) * DS])

        @pl.when(any_false(safe))
        def _():
            lax.fori_loop(0, NP * n_rb, recompute_with_max, 0)

            def project_again(r, carry):
                def normalise(p, carry):
                    p0[pl.ds(p * (PW // 8), PW // 8)] = normalised(
                        o_s[r, 2 * p], o_s[r, 2 * p + 1])[0].reshape(PW // 8, 8, RB)
                    return carry

                def token_tile(t, carry):
                    rows = _rows(r * RB + t * 128, 128)
                    ot = p0[0:D // 8, :, _rows(t * 128, 128)].reshape(D, 128)
                    y_s[rows, :] = (x_v[rows, :].astype(F32)
                                    + gate_a * _dot(ot.astype(BF16).T, wo_v[...]))
                    return carry

                lax.fori_loop(0, NP, normalise, 0)
                return lax.fori_loop(0, n_qt, token_tile, carry)

            lax.fori_loop(0, n_rb, project_again, 0)
            lax.fori_loop(0, HB // 16, lambda e, _: norm2(0, 0, e * 16), zero_s[0:8, 0:128])

        def ffn_block(r, carry):
            lu = lu_s.at[r & 1]
            tail = _unpack(tail_operand(lu))
            for p in range(n_fp - 1):
                rest = _dot(tail, wgu_v[p * 512:(p + 1) * 512, 2 * DS:], NT)
                m = [_dot(_unpack(lu[i, 0:HB // 2]), _unpack(ru_s[i, p * 128:(p + 1) * 128]), NT)
                     for i in range(7)]
                act = {}
                for a, b, combine in STRASSEN_OUT.values():
                    gu = combine(m) + rest[a * HB:(a + 1) * HB, b * 256:(b + 1) * 256]
                    act[a, b] = _geglu(gu[:, 0:128], gu[:, 128:])
                store_activations(p, act[0, 0], act[0, 1], act[1, 0], act[1, 1])
            gu = _dot(_unpack(plain_operand(lu)), wgu_v[(n_fp - 1) * 512:2 * FF], NT)
            one = _geglu(gu[:, 0:128], gu[:, 128:256])
            two = jnp.concatenate([_geglu(gu[:, 256:256 + f_tail], gu[:, 256 + f_tail:]),
                                   jnp.zeros((RB, 128 - f_tail), F32)], axis=1)
            store_activations(n_fp - 1, one[0:HB], two[0:HB], one[HB:], two[HB:])

            def write(r0, c0, y):
                rows = pl.ds(pl.multiple_of(r * RB + r0, HB), y.shape[0])
                cs = slice(c0, c0 + y.shape[1])
                out_v[rows, cs] = (y_s[rows, cs] + gate_b[:, cs] * y).astype(BF16)
                copy(out_v.at[rows, cs], out_hbm.at[rows, cs], sem_out).start()

            act = jnp.concatenate([
                jnp.concatenate([ld_s[i, :, p * 128:(p + 1) * 128]
                                 for p in range(n_fp) for i in pair], axis=1)
                for pair in ((2, 7), (8, 3))], axis=0)
            write(0, 2 * DS, _dot(_unpack(act), wd_v[:, 2 * DS:]))
            following = _jobs(lu_s, norm2, HB, jnp.minimum(r + 1, n_rb - 1), zero0 + 1 - (r & 1))
            m = {}
            for n, i in enumerate(STRASSEN_ORDER):
                m[i] = _dot(_unpack(ld_s[i]), _unpack(rd_s[i, 0:n_fp * 64]))
                paced([m[i]], following[4 * n:4 * (n + 1)])
                if i in STRASSEN_OUT:
                    a, b, combine = STRASSEN_OUT[i]
                    write(a * HB, b * DS, combine(m))
            return carry

        def store_activations(p, a11, a12, a21, a22):
            for i, v in enumerate(_strassen_lhs(a11, a12, a21, a22) + (a12, a21)):
                ld_s[i, :, p * 128:(p + 1) * 128] = _pack(v)

        lax.fori_loop(0, n_rb, ffn_block, 0)
        copy(out_v, out_hbm, sem_out).wait()

    pl.run_scoped(
        finish,
        pltpu.VMEM((2, 11, HB // 2 + 16, DS), F32),
        pltpu.VMEM((9, HB // 2, n_fp * 128), F32),
        pltpu.VMEM((3, 11, HB // 2, DS), F32),
        pltpu.VMEM((7, DS // 2 + 32, DS), F32),
        pltpu.VMEM((S, D), BF16),
        pltpu.VMEM((D, 4 * D), BF16),
        pltpu.VMEM((D, D), BF16),
    )


@jax.jit
def pallas_adaLN_cond__mha_block__geglu_ffn__prompt_kernel(
    A_x: jax.Array,
    A_wqkv: jax.Array,
    A_wo: jax.Array,
    B_x: jax.Array,
    B_w_gate: jax.Array,
    B_w_up: jax.Array,
    B_w_down: jax.Array,
    c: jax.Array,
    w_mod: jax.Array,
):
    del B_x
    B, S, D = A_x.shape
    FF = B_w_down.shape[0]
    assert (B, S, D, FF) == (1, 2048, 640, 1728)
    DH, NP, n_rb = D // H, H // 2, S // RB
    n_fp = (FF // 128 + 1) // 2
    hbm = pl.BlockSpec(memory_space=pl.ANY)
    vmem = pltpu.VMEM
    p_rows = n_rb * S // 8 + (NV // 8 + 1) * DH // (RB // 128)
    out = pl.pallas_call(
        _kernel,
        out_shape=jax.ShapeDtypeStruct((S, D), A_x.dtype),
        in_specs=[hbm] * 8,
        out_specs=hbm,
        scratch_shapes=[
            vmem((p_rows, 8, RB), F32),
            vmem((p_rows, 8, RB), F32),
            vmem((S, D), F32),
            vmem((S, D), BF16),
            vmem((D, 3 * D), BF16),
            vmem((2 * FF, D), BF16),
            vmem((n_fp * 256, D), BF16),
            vmem((D, 2 * D), BF16),
            vmem((NP, S // 2 + 32, 128), F32),
            vmem((NP, n_rb, 16, RB), F32),
            vmem((NP, n_rb, 24, RB), F32),
            vmem((NP, n_rb, 2 * DH, RB), F32),
            vmem((H, n_rb, 24, RB), F32),
            vmem((24, RB), F32),
            vmem((n_rb, H, 24, RB), F32),
            vmem((7, (n_fp - 1) * 128 + 64, DS), F32),
            vmem((7, n_fp * 64 + 32, DS), F32),
            pltpu.SemaphoreType.DMA((12,)),
        ],
        compiler_params=pltpu.CompilerParams(vmem_limit_bytes=127 * 1024 * 1024),
        name="adaln_mha_geglu_block",
    )(c, A_x.reshape(S, D), A_wqkv, A_wo, B_w_gate.T, B_w_up.T, B_w_down, w_mod)
    return out.reshape(B, S, D)
```

```python
import functools
import math

import numpy as np
import jax
import jax.numpy as jnp
import jax.experimental.pallas as pl
import jax.experimental.pallas.tpu as pltpu
from jax import lax

F32 = jnp.float32
BF16 = jnp.bfloat16

H = 32
EPS = 1e-5
RB = 512
HB = RB // 2
KC = 128
DS = 256
NV = 336
NV0 = 288
KS = 256

SUM_MIN = 2.0 ** -40
SUM_MAX = 2.0 ** 100
FINITE = float(np.finfo(np.float32).max)

NN = (((1,), (0,)), ((), ()))
NT = (((1,), (1,)), ((), ()))


def _dot(a, b, dims=NN):
    return lax.dot_general(a, b, dims, preferred_element_type=F32)


def _pack(v):
    return pltpu.bitcast(v.astype(BF16), F32)


def _unpack(v):
    return pltpu.bitcast(v, BF16)


def _rows(start, n):
    return pl.ds(pl.multiple_of(start, n), n)


def _layernorm(x):
    inv_d = 1.0 / x.shape[-1]
    xc = x - jnp.sum(x, axis=-1, keepdims=True) * inv_d
    var = jnp.sum(xc * xc, axis=-1, keepdims=True) * inv_d
    return xc * lax.rsqrt(var + EPS)


def _geglu(g, u):
    c0 = math.sqrt(2.0 / math.pi)
    t = jnp.tanh(g * (c0 + (c0 * 0.044715) * (g * g)))
    hg = 0.5 * g
    return (hg + hg * t) * u


def _strassen_lhs(a11, a12, a21, a22):
    return a11 + a22, a21 + a22, a11, a22, a11 + a12, a21 - a11, a12 - a22


def _strassen_rhs(b11, b12, b21, b22):
    return b11 + b22, b11, b12 - b22, b21 - b11, b22, b11 + b12, b21 + b22


def _token_operands(a11, a12, a21, a22, tail1, tail2):
    return _strassen_lhs(a11, a12, a21, a22) + (tail1, tail2, a12, a21)


STRASSEN_ORDER = (2, 4, 1, 3, 0, 6, 5)
STRASSEN_OUT = {
    4: (0, 1, lambda m: m[2] + m[4]),
    3: (1, 0, lambda m: m[1] + m[3]),
    6: (0, 0, lambda m: m[0] + m[3] - m[4] + m[6]),
    5: (1, 1, lambda m: m[0] - m[1] + m[2] + m[5]),
}


def _jobs(ref, fn, n, *args):
    return [(ref, functools.partial(fn, *args, e)) for e in range(0, n, 16)]


def _merge(*lists):
    keyed = [((i + 0.5) / len(l), j, v) for j, l in enumerate(lists) for i, v in enumerate(l)]
    return [v for _, _, v in sorted(keyed, key=lambda t: t[:2])]


def _kernel(c_hbm, x_hbm, wqkv_hbm, wo_hbm, wgt_hbm, wut_hbm, wd_hbm, wmod_hbm, out_hbm,
            p0, p1, y_s, x_v, wqkv_v, wgu_v, wd_v, wmod_v,
            k_s, qe_s, qo_s, qf_s, v_s, zero_s, o_s, ru_s, rd_s, sems):
    S, D = x_v.shape
    FF = wd_hbm.shape[0]
    DH = D // H
    NP = H // 2
    PW = 2 * DH
    n_rb = S // RB
    n_kc = S // KC
    n_qt = RB // 128
    n_fp = pl.cdiv(FF, 256)

    def copy(src, dst, sem):
        return pltpu.make_async_copy(src, dst, sems.at[sem])

    def cols(src, dst, lo, hi, sem):
        return copy(src.at[:, lo:hi], dst.at[:, lo:hi], sem)

    cp_x = [copy(x_hbm.at[lo * HB:hi * HB], x_v.at[lo * HB:hi * HB], sem)
            for sem, (lo, hi) in enumerate(((0, 2), (2, 3), (3, 4), (4, 6), (6, 8)))]
    cp_scale = cols(wmod_hbm, wmod_v, D, 2 * D, 5)
    cp_wk = [cols(wqkv_hbm, wqkv_v, D, D + KS, 6), cols(wqkv_hbm, wqkv_v, D + KS, 2 * D, 7)]
    cp_qv = [cols(wmod_hbm, wmod_v, 0, D, 8), cols(wqkv_hbm, wqkv_v, 0, D, 8),
             cols(wqkv_hbm, wqkv_v, 2 * D, 3 * D, 8)]
    cp_ffn = [copy(wd_hbm, wd_v.at[0:FF], 9)]
    f_main = (n_fp - 1) * 256
    for lo in list(range(0, f_main, 128)) + list(range(f_main, FF, 64)):
        n = 128 if lo < f_main else 64
        cp_ffn.append(copy(wgt_hbm.at[lo:lo + n], wgu_v.at[2 * lo:2 * lo + n], 9))
        cp_ffn.append(copy(wut_hbm.at[lo:lo + n], wgu_v.at[2 * lo + n:2 * lo + 2 * n], 9))
    sem_late, sem_out = 10, 11

    def start(c_v):
        cp_c = copy(c_hbm, c_v, 0)
        for cp in [cp_c, cp_x[0], cp_scale] + cp_wk + cp_x[1:] + cp_qv + cp_ffn:
            cp.start()
        cp_c.wait()
        cp_x[0].wait()
        return c_v[...].astype(F32)

    cc = pl.run_scoped(start, pltpu.VMEM((1, D), BF16))
    sc = jnp.broadcast_to(cc / (1.0 + jnp.exp(-cc)), (8, D))

    def hidden_zero(n):
        return ((n * (n + 1)) & 1) * n

    seed = jnp.max(cc[:, 0:128]).astype(jnp.int32)
    zero0 = hidden_zero(seed)
    marks = {}

    def paced(results, work):
        pieces = [(v, r) for v in results for r in range(0, v.shape[0], 8)]
        for i, (ref, fn) in enumerate(work):
            v, r = pieces[len(pieces) * i // len(work)]
            mark = lax.slice(v, (r, 0), (r + 8, 128))
            if ref is None:
                fn(mark)
                continue
            k = marks[id(ref)] = marks.get(id(ref), -1) + 1
            *idx, e = map(int, np.unravel_index(k, ref.shape[:-2] + (64,), order="F"))
            e = ref.shape[-2] - 8 - 8 * e
            ref[(*idx, slice(e, e + 8), slice(0, 128))] = mark
            fn()

    def tail_operand(ref):
        return jnp.concatenate(
            [ref[7 + half, 0:HB // 2, 3 * DS - D:] for half in range(2)], axis=0)

    def plain_operand(ref):
        head = jnp.concatenate([
            jnp.concatenate([ref[i, 0:HB // 2] for i in pair], axis=1)
            for pair in ((2, 9), (10, 3))], axis=0)
        return jnp.concatenate([head, tail_operand(ref)], axis=1)

    n_kb = NV // 8 * DH

    def kb_pos(i):
        return n_rb * S // 8 + i // n_qt, slice(i % n_qt * 128, (i % n_qt + 1) * 128)

    def kb_store(ref, zero, pair, odd, g, d):
        col = d + (DH if odd else 0)
        val = jnp.broadcast_to(k_s[pair, g * 4:g * 4 + 8, col:col + 1], (8, 128))
        for i, v in enumerate(lax.split(_unpack(val).astype(F32), [8, 8], 0)):
            row, cs = kb_pos((g + i) * DH + d)
            ref[lax.add(zero, np.int32(row)), :, cs] = v

    def project(xn_s, h0_s, wt_s, wqv_s, hq0_s, hq1_s, hq2_s):
        q_scale = DH ** -0.5 * math.log2(math.e)

        def norm0(r, e):
            xn = _layernorm(x_v[r * RB + 2 * e:r * RB + 2 * e + 32].astype(F32))
            xn_s[zero0 + r, 2 * e:2 * e + 32] = xn
            h0_s[r * HB + e:r * HB + e + 16] = _pack(xn * scale_a)

        def norm1(r, ref, slot, e):
            h1, h2 = (xn_s[r, half * HB + e:half * HB + e + 16] * scale_a + shift_a
                      for half in range(2))
            ops = _strassen_rhs(h1[:, 0:DS], h2[:, 0:DS], h1[:, DS:2 * DS], h2[:, DS:2 * DS])
            for i, v in enumerate(ops + (h1[:, D - DS:], h2[:, D - DS:])):
                ref[zero0 + slot, i, e // 2:e // 2 + 8] = _pack(v)

        def k_windows(start, e):
            k = _pack(y_s[_rows(2 * (start + e), 32), :] + k_shift)
            lane = lax.broadcasted_iota(jnp.int32, (16, 128), 1)
            for p in range(NP):
                t, a = divmod(p * PW, 128)
                w = k[:, t * 128:(t + 1) * 128]
                if a + PW > 128:
                    w = jnp.where(lane < a, k[:, (t + 1) * 128:(t + 2) * 128], w)
                k_s[zero0 + p, _rows(start + e, 16), :] = pltpu.roll(w, 128 - a, 1) if a else w

        def transpose_w(i, t):
            lo = 2 * i * D + t * 128
            wt = pltpu.bitcast(wqkv_v[:, lo:lo + 128].T, F32)
            for e in range(0, 128, 64):
                a, row = divmod(t * 128 + e, D // 2)
                row = (i * D // 2 + row) // 2
                wt_s[zero0 + a, row:row + 32] = wt[e // 2:e // 2 + 32]

        def prep_qv(r):
            top, bot = (_unpack(wt_s[a, r // 2:r // 2 + 8, 0:2 * DS]).astype(F32)
                        for a in range(2))
            for i, v in enumerate(_strassen_lhs(top[:, 0:DS], top[:, DS:],
                                                bot[:, 0:DS], bot[:, DS:])):
                wqv_s[zero0 + i, r // 2:r // 2 + 8] = _pack(v)

        def prep_kb(d, mark):
            row, cs = kb_pos(n_kb + d)
            p1[row, :, cs] = mark
            for g in range(0, NV0 // 8, 2):
                kb_store(p1, zero0, 0, False, g, d)

        def prep_up(p, r):
            one, two = (wgu_v[_rows(p * 512 + i * 256 + r, 16), 0:2 * DS].astype(F32)
                        for i in range(2))
            for i, v in enumerate(_strassen_rhs(one[:, 0:DS], two[:, 0:DS],
                                                one[:, DS:], two[:, DS:])):
                ru_s[zero0 + i, _rows(p * 128 + r // 2, 8), :] = _pack(v)

        def prep_up_last(half, r):
            r = half * 64 + r
            one, two = (wgu_v[_rows(2 * f_main + i * 128 + r, 16), 0:2 * DS].astype(F32)
                        for i in range(2))
            for i, v in enumerate(_strassen_rhs(one[:, 0:DS], two[:, 0:DS],
                                                one[:, DS:], two[:, DS:])):
                ru_s[zero0 + i, _rows((f_main + r) // 2, 8), :] = _pack(v)

        def prep_down(half, p, r):
            r = half * 64 + r
            one, two = (wd_v[_rows(p * 256 + i * 128 + r, 16), 0:2 * DS].astype(F32)
                        for i in range(2))
            for i, v in enumerate(_strassen_rhs(one[:, 0:DS], one[:, DS:],
                                                two[:, 0:DS], two[:, DS:])):
                rd_s[zero0 + i, _rows(p * 64 + r // 2, 8), :] = _pack(v)

        def k_part(row, n, lo, hi, work=()):
            kf = [_dot(_unpack(h0_s[i // 2:i // 2 + 64]), wqkv_v[:, D + lo:D + hi])
                  for i in range(row, row + n, 128)]
            paced(kf, work)
            for i, v in enumerate(kf):
                y_s[row + i * 128:row + (i + 1) * 128, lo:hi] = v

        def qv_emit(r, a, b, qv):
            cs = slice(b * HB, (b + 1) * HB)
            qt, vt = qv[0:D // 2] * q_scale, qv[D // 2:]
            zeros = jnp.zeros((8, HB), F32)
            even = lax.broadcasted_iota(jnp.int32, (8, HB), 0) < DH % 8
            for i in range(NP // 2):
                p, o = a * NP // 2 + i, i * PW
                q_mid, v_mid = qt[o + 16:o + 24], vt[o + 16:o + 24]
                qe_s[p, r, :, cs] = _pack(jnp.concatenate(
                    [qt[o:o + 16], jnp.where(even, q_mid, 0.0), zeros], axis=0))
                qo_s[p, r, :, cs] = _pack(jnp.concatenate(
                    [zeros, zeros, jnp.where(even, 0.0, q_mid), qt[o + 24:o + 40], zeros], axis=0))
                qf_s[p, r, :, cs] = qt[o:o + PW]
                v_s[2 * p, r, :, cs] = jnp.concatenate(
                    [vt[o:o + 16], jnp.where(even, v_mid, 1.0)], axis=0)
                v_s[2 * p + 1, r, :, cs] = jnp.concatenate(
                    [jnp.where(even, 1.0, v_mid), vt[o + 24:o + 40]], axis=0)

        def qv_block(r, hq, work, early=()):
            m, rest = {}, {}

            def last_columns(a):
                return _dot(_unpack(wt_s[a, 0:D // 2, 2 * DS:]), _unpack(tail_operand(hq)), NT)

            if early:
                rest = {a: last_columns(a) for a in range(2)}
                paced(list(rest.values()), early)
            for n, i in enumerate(STRASSEN_ORDER):
                m[i] = _dot(_unpack(wqv_s[i, 0:D // 2]), _unpack(hq[i, 0:HB // 2]), NT)
                paced([m[i]], work[len(work) * n // 7:len(work) * (n + 1) // 7])
                if i in STRASSEN_OUT:
                    a, b, combine = STRASSEN_OUT[i]
                    if a not in rest:
                        rest[a] = last_columns(a)
                    qv_emit(r, a, b, combine(m) + rest[a][:, b * HB:(b + 1) * HB])

        xn_s[0, 0:RB] = _layernorm(x_v[0:RB].astype(F32))
        cp_scale.wait()
        scale_a = 1.0 + _dot(sc, wmod_v[:, D:2 * D])[0:1]
        h0_s[0:HB] = _pack(xn_s[0, 0:RB] * scale_a)
        norm = [_jobs(xn_s, norm0, HB, r) for r in range(n_rb)]
        n = HB // 32
        cp_wk[0].wait()
        k_part(0, RB, 0, KS)
        cp_wk[1].wait()
        k_part(0, HB, KS, D)
        cp_x[1].wait()
        k_part(HB, HB, KS, D, norm[1][:n])
        cp_x[2].wait()
        k_part(RB, HB, 0, D, norm[1][n:])
        cp_x[3].wait()
        k_part(RB + HB, HB, 0, D, norm[2][:n])
        cp_x[4].wait()
        k_part(2 * RB, HB, 0, D, norm[2][n:] + norm[3][:n // 2])
        k_part(2 * RB + HB, HB, 0, D, norm[3][n // 2:])
        for cp in cp_qv:
            cp.wait()
        shift_a = _dot(sc, wmod_v[:, 0:D])
        k_part(3 * RB, HB, 0, D, [(wt_s, functools.partial(transpose_w, i, t))
                                  for i in range(2) for t in range(D // 128)])
        k_shift = _dot(shift_a, wqkv_v[:, D:2 * D])[0:1]
        shift_a = shift_a[0:1]
        prep = _jobs(wqv_s, prep_qv, D)
        k_part(3 * RB + HB, HB, 0, D,
               _merge(prep[:len(prep) // 3], _jobs(hq0_s, norm1, HB, 0, hq0_s, 0)))
        qv_block(0, hq0_s.at[0],
                 _jobs(hq1_s, norm1, HB, 1, hq1_s, 0) + _jobs(hq2_s, norm1, HB, 2, hq2_s, 0),
                 prep[len(prep) // 3:])
        qv_block(1, hq1_s.at[0], _merge(
            _jobs(hq2_s, norm1, HB, 3, hq2_s, 1),
            _jobs(k_s, k_windows, HB, 0)
            + [(None, functools.partial(prep_kb, d)) for d in range(DH)]))
        for cp in cp_ffn:
            cp.wait()
        wd_v[FF:] = jnp.zeros((wd_v.shape[0] - FF, D), BF16)

        def late_block(i, carry):
            marks.clear()
            n = (n_fp - 1) // 2
            qv_block(i + 2, hq2_s.at[i], _merge(
                [j for p in range(n) for j in _jobs(ru_s, prep_up, 256, i * n + p)]
                + _jobs(ru_s, prep_up_last, 64, i),
                [j for p in range(n_fp) for j in _jobs(rd_s, prep_down, 64, i, p)],
                _jobs(k_s, k_windows, 3 * HB // 2, HB + i * (3 * HB // 2))))
            return carry

        lax.fori_loop(0, 2, late_block, 0)

    pl.run_scoped(
        project,
        pltpu.VMEM((n_rb, RB + 96, D), F32),
        pltpu.VMEM((S // 2, D), F32),
        pltpu.VMEM((2, D // 2 + 64, D), F32),
        pltpu.VMEM((7, D // 2 + 48, DS), F32),
        pltpu.VMEM((1, 9, HB // 2 + 16, DS), F32),
        pltpu.VMEM((1, 9, HB // 2 + 16, DS), F32),
        pltpu.VMEM((2, 9, HB // 2 + 16, DS), F32),
    )

    zero_s[...] = jnp.zeros(zero_s.shape, F32)
    even_rows = lax.broadcasted_iota(jnp.int32, (8, RB), 0) < DH % 8

    def pv_tile(head, qb, c, pr, acc, dtype=F32):
        g = (qb * S + c * KC) // 8
        p = pr[g:g + KC // 8].reshape(KC, RB).astype(dtype)
        r, lo = divmod(c * KC, RB)
        return acc + _dot(v_s[head, r, :, lo:lo + KC], p)

    def phase(head, odd, pr, pw, first=False):
        zero = zero0 if first else hidden_zero(head)
        keep = lax.broadcasted_iota(jnp.int32, (8, 128), 0) >= zero
        pair1 = (head + 1) // 2
        pair2 = jnp.minimum((head + 2) // 2, NP - 1)
        q_s = qe_s if odd else qo_s
        columns = [(g, d) for d in range(DH) for g in range(0, NV // 8, 2)]
        state = {"offset": zero}

        def vector_scores(qb, g, t):
            if g == 0:
                rows = [jnp.broadcast_to(qf_s[pair1, qb, d:d + 1, t * 128:(t + 1) * 128], (8, 128))
                        for d in (range(DH) if odd else range(DH, PW))]
                state["q"] = [lax.concatenate(rows[i:i + n_qt], 1) for i in range(0, DH, n_qt)]
            state["offset"] = lax.add(state["offset"], zero)
            n = DH // n_qt
            k = pr[pl.ds(lax.add(state["offset"], np.int32(kb_pos(g * DH)[0])), n)]
            part = None
            for kv, qv in zip(lax.split(k.reshape(n * 8, RB), [8] * n, 0), state["q"]):
                prod = lax.mul(kv, qv)
                part = prod if part is None else lax.add(part, prod)
            return functools.reduce(lax.add, lax.split(part, [128] * n_qt, 1))

        for qb in range(n_rb):
            nv = NV0 if first else NV - 16 * (1 - qb % 2)
            bounds = [nv + (S - nv) // 16 * c // n_kc * 16 for c in range(n_kc + 1)]
            n_pieces = (S - nv) // 8 + (0 if first else 3 * n_kc)
            scores = [(g, t) for t in range(n_qt) for g in range(nv // 8)]
            cut = np.cumsum([0] + [1 if first or i % 2 else 4 for i in range(n_rb)])
            share = columns[len(columns) * cut[qb] // cut[-1]:len(columns) * cut[qb + 1] // cut[-1]]
            done = [0, 0, 0]

            def fill(piece):
                done[0] += 1
                while (done[1] + 0.9) * n_pieces <= done[0] * len(scores):
                    g, t = scores[done[1]]
                    done[1] += 1
                    s = lax.select(keep, vector_scores(qb, g, t),
                                   lax.slice(piece, (0, t * 128), (8, (t + 1) * 128)))
                    pw[lax.add(zero, np.int32(qb * S // 8 + g)), :, t * 128:(t + 1) * 128] = (
                        lax.exp2(s))
                while (done[2] + 0.5) * n_pieces <= done[0] * len(share):
                    kb_store(pw, zero, pair2, odd, *share[done[2]])
                    done[2] += 1

            acc = zero_s[...]
            for c in range(n_kc):
                k = k_s[pair1, bounds[c] // 2:bounds[c + 1] // 2, 0:2 * q_s.shape[2]]
                s = _dot(_unpack(k), _unpack(q_s[pair1, qb]))
                for i, piece in enumerate(lax.split(s, [8] * (s.shape[0] // 8), 0)):
                    pw[(qb * S + bounds[c]) // 8 + i] = lax.exp2(piece)
                    fill(piece)
                if not first:
                    acc = pv_tile(head, qb, c, pr, acc)
                    for piece in lax.split(acc, [8] * 3, 0):
                        fill(piece)
            assert done[1:] == [len(scores), len(share)]
            if not first:
                o_s[qb, head] = acc

    def normalised(even, odd):
        total = jnp.where(even_rows, odd[0:8], even[16:24])
        inv = pl.reciprocal(total, approx=True)
        inv = inv * (2.0 - total * inv)
        inv_even, inv_odd = inv[7:8], inv[0:1]
        mid = (jnp.where(even_rows, even[16:24], odd[0:8])
               * jnp.where(even_rows, inv_even, inv_odd))
        return jnp.concatenate([even[0:16] * inv_even, mid, odd[8:24] * inv_odd], axis=0), total

    def in_range(pairs):
        check = functools.reduce(jnp.add, [o[e:e + 8] for o, _ in pairs for e in range(0, PW, 8)])
        totals = [total for _, total in pairs]
        return ((jnp.abs(check) <= FINITE)
                & (functools.reduce(jnp.minimum, totals) >= SUM_MIN)
                & (functools.reduce(jnp.maximum, totals) <= SUM_MAX))

    def any_false(flags):
        return jnp.min(jnp.where(functools.reduce(jnp.logical_and, flags), 1.0, 0.0)) == 0.0

    def recompute_with_max(i, carry):
        pair, qb = i // n_rb, i % n_rb

        @pl.when(any_false([in_range([normalised(o_s[qb, 2 * pair], o_s[qb, 2 * pair + 1])])]))
        def _():
            for head, q_s in ((2 * pair, qe_s), (2 * pair + 1, qo_s)):
                def scores(r):
                    return _dot(_unpack(k_s[pair, _rows(r * HB, HB), 0:2 * q_s.shape[2]]),
                                _unpack(q_s[pair, qb]))

                top = lax.fori_loop(
                    0, n_rb,
                    lambda r, m: jnp.maximum(m, jnp.max(scores(r), axis=0, keepdims=True)),
                    jnp.full((1, RB), -jnp.inf, F32))
                o_s[qb, head] = lax.fori_loop(
                    0, n_rb,
                    lambda r, acc: acc + _dot(v_s[head, r],
                                              jnp.exp2(scores(r) - top).astype(BF16)),
                    jnp.zeros((24, RB), F32))
        return carry

    def finish(lu_s, ld_s, lo_s, ro_s, out_v, wmodb_v, wo_v):
        marks.clear()
        cp_late = [copy(wmod_hbm.at[:, 2 * D:], wmodb_v, sem_late), copy(wo_hbm, wo_v, sem_late)]

        def head_pair(pair, carry):
            phase(2 * pair, False, p0, p1)

            @pl.when(pair < NP - 1)
            def _():
                phase(2 * pair + 1, True, p1, p0)

            @pl.when(pair == 1)
            def _():
                for cp in cp_late:
                    cp.start()
            return carry

        phase(-1, True, p1, p0, first=True)
        lax.fori_loop(0, NP, head_pair, 0)
        for cp in cp_late:
            cp.wait()

        def last_head(qb, n):
            acc = zero_s[...]
            for c in range(n_kc):
                acc = pv_tile(H - 1, qb, c, p1, acc, BF16)
                if c == n_kc - 1:
                    o_s[qb, H - 1] = acc
                if (c + 1) * n // n_kc > c * n // n_kc:
                    yield acc

        def prep_wo(r):
            one, two = (wo_v[i * DS + r:i * DS + r + 16, 0:2 * DS].astype(F32) for i in range(2))
            for i, v in enumerate(_strassen_rhs(one[:, 0:DS], one[:, DS:],
                                                two[:, 0:DS], two[:, DS:])):
                ro_s[zero0 + i, r // 2:r // 2 + 8] = _pack(v)

        def norm2(r, slot, e):
            h1, h2 = (_layernorm(y_s[_rows(r * RB + half * HB + e, 16), :]) * scale_b + shift_b
                      for half in range(2))
            ops = [_pack(v) for v in _token_operands(
                h1[:, 0:DS], h1[:, DS:2 * DS], h2[:, 0:DS], h2[:, DS:2 * DS],
                h1[:, D - DS:], h2[:, D - DS:])]
            for i, v in enumerate(ops):
                lu_s[slot, i, _rows(e // 2, 8), :] = v
            return ops[0][:, 0:128]

        accs, mod = [], []
        for i, acc in enumerate(last_head(0, 4)):
            accs.append(acc)
            mod.append(_dot(sc, wmodb_v[:, i * D:(i + 1) * D])[0:1])
        paced(accs, _jobs(ro_s, prep_wo, DS))
        gate_a, shift_b, scale_b, gate_b = mod
        scale_b = 1.0 + scale_b

        safe = []
        for r in range(n_rb):
            steps = last_head(r + 1, 8) if r + 1 < n_rb else iter(range(8))
            pairs = [normalised(o_s[r, 2 * p], o_s[r, 2 * p + 1]) for p in range(NP)]
            safe.append(in_range(pairs))
            ot = jnp.concatenate([o for o, _ in pairs], axis=0)
            for i, v in enumerate(_token_operands(
                    ot[0:DS, 0:HB], ot[DS:2 * DS, 0:HB], ot[0:DS, HB:], ot[DS:2 * DS, HB:],
                    ot[2 * DS:, 0:HB], ot[2 * DS:, HB:])):
                lo_s[r % 2, i, :, DS - v.shape[0]:] = pltpu.bitcast(v.astype(BF16).T, F32)
            lo = lo_s.at[r % 2]

            def add_attention(r0, c0, y):
                rows = slice(r * RB + r0, r * RB + r0 + y.shape[0])
                cs = slice(c0, c0 + y.shape[1])
                y_s[rows, cs] = x_v[rows, cs].astype(F32) + gate_a[:, cs] * y

            next(steps)
            rest = _dot(_unpack(tail_operand(lo)), wo_v[2 * DS:, 0:2 * DS])
            add_attention(0, 2 * DS, _dot(_unpack(plain_operand(lo)), wo_v[:, 2 * DS:]))
            m = {}
            for n, i in enumerate(STRASSEN_ORDER):
                next(steps)
                m[i] = _dot(_unpack(lo[i]), _unpack(ro_s[i, 0:DS // 2]))
                k = HB // 16 + 1 - (n_rb - r) * len(STRASSEN_ORDER) + n
                if 0 <= k < HB // 16:
                    lo_s[zero0 + 2, k // 8, k % 8 * 8:k % 8 * 8 + 8, 0:128] = norm2(0, 0, k * 16)
                if i in STRASSEN_OUT:
                    a, b, combine = STRASSEN_OUT[i]
                    add_attention(a * HB, b * DS,
                                  combine(m) + rest[a * HB:(a + 1) * HB, b * DS:(b + 1) * DS])

        @pl.when(any_false(safe))
        def _():
            lax.fori_loop(0, NP * n_rb, recompute_with_max, 0)

            def project_again(r, carry):
                def normalise(p, carry):
                    p0[pl.ds(p * (PW // 8), PW // 8)] = normalised(
                        o_s[r, 2 * p], o_s[r, 2 * p + 1])[0].reshape(PW // 8, 8, RB)
                    return carry

                def token_tile(t, carry):
                    rows = _rows(r * RB + t * 128, 128)
                    ot = p0[0:D // 8, :, _rows(t * 128, 128)].reshape(D, 128)
                    y_s[rows, :] = (x_v[rows, :].astype(F32)
                                    + gate_a * _dot(ot.astype(BF16).T, wo_v[...]))
                    return carry

                lax.fori_loop(0, NP, normalise, 0)
                return lax.fori_loop(0, n_qt, token_tile, carry)

            lax.fori_loop(0, n_rb, project_again, 0)
            lax.fori_loop(0, HB // 16, lambda e, _: norm2(0, 0, e * 16), zero_s[0:8, 0:128])

        def store_activations(p, a11, a12, a21, a22):
            for i, v in enumerate(_strassen_lhs(a11, a12, a21, a22) + (a12, a21)):
                ld_s[i, :, p * 128:(p + 1) * 128] = _pack(v)

        def ffn_block(r, carry):
            marks.clear()
            lu = lu_s.at[r & 1]
            tail = _unpack(tail_operand(lu))
            for p in range(n_fp - 1):
                rest = _dot(tail, wgu_v[p * 512:(p + 1) * 512, 2 * DS:], NT)
                m = [_dot(_unpack(lu[i, 0:HB // 2]), _unpack(ru_s[i, p * 128:(p + 1) * 128]), NT)
                     for i in range(7)]
                act = {}
                for a, b, combine in STRASSEN_OUT.values():
                    gu = combine(m) + rest[a * HB:(a + 1) * HB, b * 256:(b + 1) * 256]
                    act[a, b] = _geglu(gu[:, 0:128], gu[:, 128:])
                store_activations(p, act[0, 0], act[0, 1], act[1, 0], act[1, 1])
            rest = _dot(tail, wgu_v[2 * f_main:2 * f_main + 256, 2 * DS:], NT)
            m = [_dot(_unpack(lu[i, 0:HB // 2]), _unpack(ru_s[i, f_main // 2:f_main // 2 + 64]), NT)
                 for i in range(7)]
            act = {}
            for a, b, combine in STRASSEN_OUT.values():
                gu = combine(m) + rest[a * HB:(a + 1) * HB, b * 128:(b + 1) * 128]
                act[a, b] = _geglu(gu[:, 0:64], gu[:, 64:])
            gu = _dot(_unpack(plain_operand(lu)), wgu_v[2 * f_main + 256:], NT)
            last = jnp.concatenate(
                [_geglu(gu[:, 0:64], gu[:, 64:]), jnp.zeros((RB, 64), F32)], axis=1)
            store_activations(
                n_fp - 1, jnp.concatenate([act[0, 0], act[0, 1]], axis=1), last[0:HB],
                jnp.concatenate([act[1, 0], act[1, 1]], axis=1), last[HB:])

            def write(r0, c0, y):
                rows = pl.ds(pl.multiple_of(r * RB + r0, HB), y.shape[0])
                cs = slice(c0, c0 + y.shape[1])
                out_v[rows, cs] = (y_s[rows, cs] + gate_b[:, cs] * y).astype(BF16)
                copy(out_v.at[rows, cs], out_hbm.at[rows, cs], sem_out).start()

            act = jnp.concatenate([
                jnp.concatenate([ld_s[i, :, p * 128:(p + 1) * 128]
                                 for p in range(n_fp) for i in pair], axis=1)
                for pair in ((2, 7), (8, 3))], axis=0)
            write(0, 2 * DS, _dot(_unpack(act), wd_v[:, 2 * DS:]))
            following = _jobs(lu_s, norm2, HB, jnp.minimum(r + 1, n_rb - 1), zero0 + 1 - (r & 1))
            m = {}
            for n, i in enumerate(STRASSEN_ORDER):
                m[i] = _dot(_unpack(ld_s[i]), _unpack(rd_s[i, 0:n_fp * 64]))
                paced([m[i]], following[len(following) * n // 6:len(following) * (n + 1) // 6])
                if i in STRASSEN_OUT:
                    a, b, combine = STRASSEN_OUT[i]
                    write(a * HB, b * DS, combine(m))
            return carry

        lax.fori_loop(0, n_rb, ffn_block, 0)
        copy(out_v, out_hbm, sem_out).wait()

    pl.run_scoped(
        finish,
        pltpu.VMEM((2, 11, HB // 2 + 16, DS), F32),
        pltpu.VMEM((9, HB // 2, n_fp * 128), F32),
        pltpu.VMEM((3, 11, HB // 2, DS), F32),
        pltpu.VMEM((7, DS // 2 + 32, DS), F32),
        pltpu.VMEM((S, D), BF16),
        pltpu.VMEM((D, 4 * D), BF16),
        pltpu.VMEM((D, D), BF16),
    )


@jax.jit
def pallas_adaLN_cond__mha_block__geglu_ffn__prompt_kernel(
    A_x: jax.Array,
    A_wqkv: jax.Array,
    A_wo: jax.Array,
    B_x: jax.Array,
    B_w_gate: jax.Array,
    B_w_up: jax.Array,
    B_w_down: jax.Array,
    c: jax.Array,
    w_mod: jax.Array,
):
    del B_x
    B, S, D = A_x.shape
    FF = B_w_down.shape[0]
    assert (B, S, D, FF) == (1, 2048, 640, 1728)
    DH, NP, n_rb = D // H, H // 2, S // RB
    n_fp = (FF // 128 + 1) // 2
    hbm = pl.BlockSpec(memory_space=pl.ANY)
    vmem = pltpu.VMEM
    p_rows = n_rb * S // 8 + (NV // 8 + 1) * DH // (RB // 128)
    out = pl.pallas_call(
        _kernel,
        out_shape=jax.ShapeDtypeStruct((S, D), A_x.dtype),
        in_specs=[hbm] * 8,
        out_specs=hbm,
        scratch_shapes=[
            vmem((p_rows, 8, RB), F32),
            vmem((p_rows, 8, RB), F32),
            vmem((S, D), F32),
            vmem((S, D), BF16),
            vmem((D, 3 * D), BF16),
            vmem((2 * FF, D), BF16),
            vmem((n_fp * 256, D), BF16),
            vmem((D, 2 * D), BF16),
            vmem((NP, S // 2 + 32, 128), F32),
            vmem((NP, n_rb, 16, RB), F32),
            vmem((NP, n_rb, 24, RB), F32),
            vmem((NP, n_rb, 2 * DH, RB), F32),
            vmem((H, n_rb, 24, RB), F32),
            vmem((24, RB), F32),
            vmem((n_rb, H, 24, RB), F32),
            vmem((7, n_fp * 128, DS), F32),
            vmem((7, n_fp * 64 + 32, DS), F32),
            pltpu.SemaphoreType.DMA((12,)),
        ],
        compiler_params=pltpu.CompilerParams(vmem_limit_bytes=127 * 1024 * 1024),
        name="adaln_mha_geglu_block",
    )(c, A_x.reshape(S, D), A_wqkv, A_wo, B_w_gate.T, B_w_up.T, B_w_down, w_mod)
    return out.reshape(B, S, D)
```
